```python
import jax
import jax.numpy as jnp

def _softmax(x, axis=-1):
    return jax.nn.softmax(x, axis=axis)
def _gelu(x):
    return jax.nn.gelu(x, approximate=True)
def _silu(x):
    return jax.nn.silu(x)
def _sigmoid(x):
    return jax.nn.sigmoid(x)
def _layernorm(x, axis=-1, eps=1e-5):
    m = jnp.mean(x, axis=axis, keepdims=True)
    v = jnp.var(x, axis=axis, keepdims=True)
    return (x - m) / jnp.sqrt(v + eps)
def _scatter_add(tgt, idx, src, axis=0):
    return tgt.at[idx].add(src)
def _segment_sum(src, seg, n):
    return jax.ops.segment_sum(src, seg, n)
class _Rng:
    def __init__(self, key):
        self._k = key
    def _next(self):
        self._k, sub = jax.random.split(self._k)
        return sub
    def normal(self, shape):
        return jax.random.normal(self._next(), shape, dtype=jnp.bfloat16)
    def randint(self, lo, hi, shape):
        return jax.random.randint(self._next(), shape, lo, hi, dtype=jnp.int32)
    def uniform(self, shape, lo=0.0, hi=1.0):
        return jax.random.uniform(self._next(), shape, jnp.bfloat16, lo, hi)
    def permutation(self, n):
        return jax.random.permutation(self._next(), n)


kernel_name = 'parallel_sum__sliding_local_dilated__glu_gated_bilinear__prompt'

def setup_inputs():
    _rng = _Rng(jax.random.key(int.from_bytes(__import__("os").urandom(4), "little")))
    _w = (lambda a: (lambda t: t.astype(jnp.bfloat16) if jnp.issubdtype(t.dtype, jnp.floating) else t)(jnp.asarray(a)))
    def _A_setup():
        B, S, D = 1, 2048, 1024
        return {
            "x": _w((lambda *s: _rng.normal(s) * 0.05)(B, S, D)),
            "wqkv": _w((lambda *s: _rng.normal(s) * 0.05)(D, 3 * D)),
            "wo": _w((lambda *s: _rng.normal(s) * 0.05)(D, D)),
        }
    _A_in = _A_setup()

    def _B_setup():
        B, S, D, F = 1, 2048, 1024, 3584
        return {
            "x": _w((lambda *s: _rng.normal(s) * 0.05)(B, S, D)),
            "w_gate": _w((lambda *s: _rng.normal(s) * 0.05)(D, F) * (D ** -0.5)),
            "w_up": _w((lambda *s: _rng.normal(s) * 0.05)(D, F) * (D ** -0.5)),
            "w_down": _w((lambda *s: _rng.normal(s) * 0.05)(F, D) * (F ** -0.5)),
        }
    _B_in = _B_setup()

    return {
        "A_x": _A_in["x"],
        "A_wqkv": _A_in["wqkv"],
        "A_wo": _A_in["wo"],
        "B_x": _B_in["x"],
        "B_w_gate": _B_in["w_gate"],
        "B_w_up": _B_in["w_up"],
        "B_w_down": _B_in["w_down"],
    }

def reference(A_x, A_wqkv, A_wo, B_x, B_w_gate, B_w_up, B_w_down):
    def _A_ref(x, wqkv, wo):
        B, S, D = x.shape
        H = 32; Dh = D // H
        W, dil = 8, 2
        qkv = (lambda x, *d: x.transpose(*d))((x @ wqkv).reshape(B, S, 3, H, Dh), 2, 0, 3, 1, 4)
        q, k, v = qkv[0], qkv[1], qkv[2]
        scale = Dh ** -0.5
        pos = jnp.arange(S)
        off = jnp.arange(W) * dil
        idx = pos[:, None] - off[None, :]
        mask = idx >= 0
        idx_c = jnp.where(mask, idx, 0).reshape(-1)
        kg = k[:, :, idx_c, :].reshape(B, H, S, W, Dh)
        vg = v[:, :, idx_c, :].reshape(B, H, S, W, Dh)
        logits = jnp.einsum("bhsd,bhswd->bhsw", q, kg) * scale
        logits = jnp.where(mask[None, None, :, :], logits, -1e9)
        attn = _softmax(logits, axis=-1)
        o = jnp.einsum("bhsw,bhswd->bhsd", attn, vg)
        return (lambda x, *d: x.transpose(*d))(o, 0, 2, 1, 3).reshape(B, S, D) @ wo

    def _B_ref(x, w_gate, w_up, w_down):
        g = jnp.einsum("bsd,df->bsf", x, w_gate)
        u = jnp.einsum("bsd,df->bsf", x, w_up)
        h = g * u
        return jnp.einsum("bsf,fd->bsd", h, w_down)

    x = A_x
    xn = _layernorm(x, axis=-1)
    return x + _A_ref(xn, A_wqkv, A_wo) + _B_ref(xn, B_w_gate, B_w_up, B_w_down)
```

```python
import functools
import contextlib
import jax
import jax.numpy as jnp
from jax import lax
import jax.experimental.pallas as pl
import jax.experimental.pallas.tpu as pltpu

S, D, F = 2048, 1024, 3584
H, DH, W, DIL = 32, 32, 8, 2
HALO = 16
NT_DIMS = (((1,), (1,)), ((), ()))
BF = jnp.bfloat16
F32 = jnp.float32
I32 = jnp.int32
R = 8


def bits(x):
    return lax.bitcast_convert_type(x, I32)


def unbits(x):
    return lax.bitcast_convert_type(x, F32)


def scope(name, on):
    return jax.named_scope(name) if on else contextlib.nullcontext()


def make_kernel(TM=224, M0=256, FC=512, last_chunk=6, prof=False):
    NS = (S - M0) // TM
    assert M0 + NS * TM == S
    NT = NS + 1
    NCH = F // FC
    TMAX = max(TM, M0)
    NB0 = M0 // R
    BPI = -(-NB0 // NCH)
    KH = D // 2
    SX, SQ, SO, SF = 0, NT, NT + 6, NT + 7
    NSEM = SF + 3 * NCH

    def attn_rows(qkv, o_scr, r0, masked, dep):
        lane = lax.broadcasted_iota(jnp.int32, (R, 128), 1)
        b0 = (lane & 1) == 0
        b1 = (lane & 2) == 0
        accs = [None] * W
        for c in range(8):
            q = qkv[0, c, pl.ds(HALO + r0, R), :]
            if c == 0 and dep is not None:
                q = unbits(bits(q) | dep)
            for w in range(W):
                t = q * qkv[1, c, pl.ds(HALO + r0 - DIL * w, R), :]
                accs[w] = t if accs[w] is None else accs[w] + t
        logits = []
        for w in range(W):
            acc = accs[w]
            acc = acc + jnp.where(b0, pltpu.roll(acc, 127, 1), pltpu.roll(acc, 1, 1))
            acc = acc + jnp.where(b1, pltpu.roll(acc, 126, 1), pltpu.roll(acc, 2, 1))
            lg = acc * (DH ** -0.5)
            if masked and w > 0:
                row = lax.broadcasted_iota(jnp.int32, (R, 128), 0) + r0
                lg = jnp.where(row >= DIL * w, lg, -1e9)
            logits.append(lg)
        m = logits[0]
        for w in range(1, W):
            m = jnp.maximum(m, logits[w])
        ps = [jnp.exp(l - m) for l in logits]
        s = ps[0]
        for w in range(1, W):
            s = s + ps[w]
        inv = 1.0 / s
        ps = [p * inv for p in ps]
        for c in range(8):
            o = None
            for w in range(W):
                t = ps[w] * qkv[2, c, pl.ds(HALO + r0 - DIL * w, R), :]
                o = t if o is None else o + t
            o_scr[pl.ds(r0, R), pl.ds(128 * c, 128)] = o.astype(o_scr.dtype)

    def kernel(x_hbm, wqkv_hbm, wo_hbm, wg_hbm, wu_hbm, wd_hbm, out_hbm,
               x_scr, out_scr, xa, xb, acc_scr, wqkv_raw, wo_raw, wt, wo_p, wg, wu, wd,
               qkv, o_scr, sem, osem):

        def tile_rows(t):
            if isinstance(t, int) and t == 0:
                return 0, M0
            start = M0 + (t - 1) * TM
            if not isinstance(start, int):
                start = pl.multiple_of(start, 16)
            return start, TM

        def x_copy(t):
            st, n = tile_rows(t)
            return pltpu.make_async_copy(x_hbm.at[pl.ds(st, n), :], x_scr.at[pl.ds(st, n), :], sem.at[SX + t])

        def out_copy(t):
            st, n = tile_rows(t)
            return pltpu.make_async_copy(out_scr.at[pl.ds(st, n), :], out_hbm.at[pl.ds(st, n), :], osem.at[t])

        def sec_copy(i):
            s, hf = i // 2, i % 2
            return pltpu.make_async_copy(wqkv_hbm.at[pl.ds(hf * KH, KH), pl.ds(s * D, D)], wqkv_raw.at[i], sem.at[SQ + i])

        def wo_copy():
            return pltpu.make_async_copy(wo_hbm, wo_raw, sem.at[SO])

        def ffn_copies(j):
            return [
                pltpu.make_async_copy(wg_hbm.at[:, pl.ds(j * FC, FC)], wg.at[j], sem.at[SF + 3 * j]),
                pltpu.make_async_copy(wu_hbm.at[:, pl.ds(j * FC, FC)], wu.at[j], sem.at[SF + 3 * j + 1]),
                pltpu.make_async_copy(wd_hbm.at[pl.ds(j * FC, FC), :], wd.at[j], sem.at[SF + 3 * j + 2]),
            ]

        def ln_rows(st, n, dst, dst_r, gate, zero):
            xr = x_scr[pl.ds(st, n), :]
            if gate is not None:
                xi = pltpu.bitcast(xr, I32)
                xi = jnp.concatenate([xi[:, 0:128] | gate, xi[:, 128:]], axis=1)
                xr = pltpu.bitcast(xi, BF)
            x = xr.astype(F32)
            mu = jnp.mean(x, axis=-1, keepdims=True)
            xc = x - mu
            var = jnp.mean(xc * xc, axis=-1, keepdims=True)
            y = (xc * lax.rsqrt(var + 1e-5)).astype(BF)
            dst[dst_r:dst_r + n, :] = y
            if zero is None:
                return None
            pk = pltpu.bitcast(y, I32)
            d = None
            for c in range(8):
                p = pk[:, 128 * c:128 * (c + 1)]
                d = p if d is None else d | p
            return d & zero

        def make_perm():
            rr = lax.broadcasted_iota(jnp.int32, (128, 128), 0)
            cc = lax.broadcasted_iota(jnp.int32, (128, 128), 1)
            src = 32 * ((rr % 16) // 4) + 4 * (rr // 16) + rr % 4
            return jnp.where(cc == src, 1.0, 0.0).astype(BF)

        def ffn_events(g, u, dn):
            return [g[0:R, 0:128], g[0:R, 384:512], u[0:R, 256:384], dn[0:R, 256:384], dn[0:R, 896:1024]]

        def first_tile():
            qkv[...] = jnp.zeros(qkv.shape, F32)
            with scope('x0wait', prof):
                x_copy(0).wait()
            ln_rows(0, M0, xa, 0, None, None)

            def qkv_body(i, carry):
                s = i // 2
                koff = pl.multiple_of((i % 2) * KH, KH)
                with scope('secwait', prof):
                    sec_copy(i).wait()
                perm = make_perm()
                for c in range(8):
                    r = lax.dot_general(perm, wqkv_raw[i, :, c * 128:(c + 1) * 128], NT_DIMS,
                                        preferred_element_type=F32).astype(BF)
                    for cp in range(8):
                        wt[s, pl.ds(128 * cp + 16 * c, 16), pl.ds(koff, KH)] = r[16 * cp:16 * cp + 16, :]
                r = lax.dot_general(xa[0:M0, pl.ds(koff, KH)], wt[s, :, pl.ds(koff, KH)], NT_DIMS,
                                    preferred_element_type=F32)
                for c in range(8):
                    qkv[s, c, HALO:HALO + M0, :] += r[:, c * 128:(c + 1) * 128]
                return carry
            with scope('f_qkv', prof):
                lax.fori_loop(0, 6, qkv_body, 0)

            for c in range(8):
                qkv[2, c, 0:HALO, :] = jnp.broadcast_to(qkv[2, c, HALO:HALO + 1, :], (HALO, 128))
            acc_scr[0:M0, :] = x_scr[0:M0, :].astype(F32)

            def ffn_body(j, carry):
                with scope('ffnwait', prof):
                    for cp in ffn_copies(j):
                        cp.wait()
                xn = xa[0:M0, :]
                g = jnp.dot(xn, wg[j], preferred_element_type=F32)
                u = jnp.dot(xn, wu[j], preferred_element_type=F32)
                h = (g * u).astype(BF)
                dn = jnp.dot(h, wd[j], preferred_element_type=F32)
                acc_scr[0:M0, :] += dn
                zvec = jnp.full((R, 128), j >> 10, I32)
                evs = [None, g[0:R, 0:128], g[0:R, 384:512], u[0:R, 0:128], u[0:R, 384:512]]
                for b in range(BPI):
                    blk = jnp.minimum(j * BPI + b, NB0 - 1)
                    e = evs[b]
                    attn_rows(qkv, o_scr, pl.multiple_of(blk * R, R), True,
                              None if e is None else bits(e) & zvec)
                return carry
            with scope('f_ffn', prof):
                lax.fori_loop(0, NCH, ffn_body, 0)

            wo_copy().wait()
            x_copy(1).wait()
            perm = make_perm()
            for c in range(8):
                r = jnp.dot(perm, wo_raw[c * 128:(c + 1) * 128, :], preferred_element_type=F32).astype(BF)
                for cp in range(8):
                    wo_p[pl.ds(128 * cp + 16 * c, 16), :] = r[16 * cp:16 * cp + 16, :]
            ln_rows(M0, TM, xa, 0, None, None)
            acc = acc_scr[0:M0, :] + jnp.dot(o_scr[0:M0, :], wo_p[...], preferred_element_type=F32)
            out_scr[0:M0, :] = acc.astype(BF)
            out_copy(0).start()
            qkv[1:3, :, 0:HALO, :] = qkv[1:3, :, M0:M0 + HALO, :]

        def steady(t):
            row0, _ = tile_rows(t)
            rown, _ = tile_rows(jnp.minimum(t + 1, NT - 1))

            @pl.when(t + 1 < NT)
            def _():
                x_copy(t + 1).wait()
            zvec = jnp.full((R, 128), t >> 10, I32)

            xn = xa[0:TM, :]
            for s in range(3):
                r = lax.dot_general(xn, wt[s], NT_DIMS, preferred_element_type=F32)
                for c in range(8):
                    qkv[s, c, HALO:HALO + TM, :] = r[:, c * 128:(c + 1) * 128]
            blocks = list(range(0, TM, R))
            nb = len(blocks)
            nuse = last_chunk
            pend = None
            acc = x_scr[pl.ds(row0, TM), :].astype(F32)
            for j in range(NCH):
                g = jnp.dot(xn, wg[j], preferred_element_type=F32)
                u = jnp.dot(xn, wu[j], preferred_element_type=F32)
                h = (g * u).astype(BF)
                dn = jnp.dot(h, wd[j], preferred_element_type=F32)
                acc = acc + dn
                if j < nuse:
                    lo = j * nb // nuse
                    hi = (j + 1) * nb // nuse
                    evs = ffn_events(g, u, dn)
                    assert hi - lo <= len(evs)
                    if hi - lo == 4:
                        evs = [evs[0], evs[2], evs[3], evs[4]]
                    for e, r0 in zip(evs, blocks[lo:hi]):
                        ed = bits(e) & zvec
                        if r0 % 16 == 0:
                            pend = ln_rows(rown + r0, 16, xb, r0, ed, zvec)
                            attn_rows(qkv, o_scr, r0, False, ed)
                        else:
                            attn_rows(qkv, o_scr, r0, False, ed | pend)
            acc = acc + jnp.dot(o_scr[0:TM, :], wo_p[...], preferred_element_type=F32)
            out_scr[pl.ds(row0, TM), :] = acc.astype(BF)
            out_copy(t).start()
            xa[0:TM, :] = xb[...]
            qkv[1:3, :, 0:HALO, :] = qkv[1:3, :, TM:TM + HALO, :]

        x_copy(0).start()
        for i in range(6):
            sec_copy(i).start()
        for j in range(NCH):
            if j == NCH - 1:
                x_copy(1).start()
            for cp in ffn_copies(j):
                cp.start()
        wo_copy().start()
        for t in range(2, NT):
            x_copy(t).start()

        with scope('first', prof):
            first_tile()

        def body(t, carry):
            with scope('steady', prof):
                steady(t)
            return carry
        lax.fori_loop(1, NT, body, 0)

        for t in range(NT):
            out_copy(t).wait()

    @jax.jit
    def run(A_x, A_wqkv, A_wo, B_x, B_w_gate, B_w_up, B_w_down):
        x = A_x.reshape(S, D)
        any_spec = pl.BlockSpec(memory_space=pl.ANY)
        out = pl.pallas_call(
            kernel,
            in_specs=[any_spec] * 6,
            out_specs=any_spec,
            out_shape=jax.ShapeDtypeStruct((S, D), BF),
            scratch_shapes=[
                pltpu.VMEM((S, D), BF), pltpu.VMEM((S, D), BF),
                pltpu.VMEM((TMAX, D), BF), pltpu.VMEM((TM, D), BF),
                pltpu.VMEM((TMAX, D), F32),
                pltpu.VMEM((6, KH, D), BF), pltpu.VMEM((D, D), BF),
                pltpu.VMEM((3, D, D), BF), pltpu.VMEM((D, D), BF),
                pltpu.VMEM((NCH, D, FC), BF), pltpu.VMEM((NCH, D, FC), BF), pltpu.VMEM((NCH, FC, D), BF),
                pltpu.VMEM((3, 8, TMAX + HALO, 128), F32),
                pltpu.VMEM((TMAX, D), BF),
                pltpu.SemaphoreType.DMA((NSEM,)), pltpu.SemaphoreType.DMA((NT,)),
            ],
            compiler_params=pltpu.CompilerParams(vmem_limit_bytes=110 << 20),
            name="fused",
        )(x, A_wqkv, A_wo, B_w_gate, B_w_up, B_w_down)
        return out.reshape(1, S, D)

    return run


_run = make_kernel()


@jax.jit
def pallas_parallel_sum__sliding_local_dilated__glu_gated_bilinear__prompt_kernel(
    A_x: jax.Array,
    A_wqkv: jax.Array,
    A_wo: jax.Array,
    B_x: jax.Array,
    B_w_gate: jax.Array,
    B_w_up: jax.Array,
    B_w_down: jax.Array,
):
    return _run(A_x, A_wqkv, A_wo, B_x, B_w_gate, B_w_up, B_w_down)
```

```python
import functools
import contextlib
import jax
import jax.numpy as jnp
from jax import lax
import jax.experimental.pallas as pl
import jax.experimental.pallas.tpu as pltpu

S, D, F = 2048, 1024, 3584
H, DH, W, DIL = 32, 32, 8, 2
HALO = 16
NT_DIMS = (((1,), (1,)), ((), ()))
BF = jnp.bfloat16
F32 = jnp.float32
I32 = jnp.int32
U32 = jnp.uint32
R = 8
PITCH = 17


def bits(x):
    return lax.bitcast_convert_type(x, I32)


def unbits(x):
    return lax.bitcast_convert_type(x, F32)


def scope(name, on):
    return jax.named_scope(name) if on else contextlib.nullcontext()


def make_kernel(TM=224, M0=256, FC=512, last_chunk=5, GM=1, LNSPAN=24, lnmode='free', xfirst=False, fev=0, nobc=False, prof=False):
    NS = (S - M0) // TM
    assert M0 + NS * TM == S
    NT = NS + 1
    NCH = F // FC
    TMAX = max(TM, M0)
    NB0 = M0 // R
    BPI = -(-NB0 // NCH)
    KH = D // 2
    SX, SQ, SO, SF = 0, NT, NT + 6, NT + 7
    NSEM = SF + 3 * NCH

    def attn_rows(qkv, o_scr, r0, masked, dep):
        lane = lax.broadcasted_iota(jnp.int32, (R, 128), 1)
        b0 = (lane & 1) == 0
        accs = [None] * W
        for c in range(8):
            q = qkv[0, c, pl.ds(HALO + r0, R), :]
            if c == 0 and dep is not None:
                q = unbits(bits(q) | dep)
            for w in range(W):
                t = q * qkv[1, c, pl.ds(HALO + r0 - DIL * w, R), :]
                accs[w] = t if accs[w] is None else accs[w] + t
        logits = []
        for w in range(W):
            acc = accs[w]
            acc = acc + pltpu.roll(acc, 64, 1)
            acc = acc + jnp.where(b0, pltpu.roll(acc, 127, 1), pltpu.roll(acc, 1, 1))
            lg = acc * (DH ** -0.5)
            if masked and w > 0:
                row = lax.broadcasted_iota(jnp.int32, (R, 128), 0) + r0
                lg = jnp.where(row >= DIL * w, lg, -1e9)
            logits.append(lg)
        m = logits[0]
        for w in range(1, W):
            m = jnp.maximum(m, logits[w])
        ps = [jnp.exp(l - m) for l in logits]
        s = ps[0]
        for w in range(1, W):
            s = s + ps[w]
        inv = 1.0 / s
        ps = [p * inv for p in ps]
        for c in range(8):
            o = None
            for w in range(W):
                t = ps[w] * qkv[2, c, pl.ds(HALO + r0 - DIL * w, R), :]
                o = t if o is None else o + t
            o_scr[pl.ds(r0, R), pl.ds(128 * c, 128)] = o.astype(o_scr.dtype)

    def kernel(x_hbm, wqkv_hbm, wo_hbm, wg_hbm, wu_hbm, wd_hbm, out_hbm,
               x_scr, out_scr, xa, xb, acc_scr, wqkv_raw, wo_raw, wta, wtb, wo_p, wg, wu, wd,
               qkv, o_scr, scru, sem, osem):

        def tile_rows(t):
            if isinstance(t, int) and t == 0:
                return 0, M0
            start = M0 + (t - 1) * TM
            if not isinstance(start, int):
                start = pl.multiple_of(start, 16)
            return start, TM

        def x_copy(t):
            st, n = tile_rows(t)
            return pltpu.make_async_copy(x_hbm.at[pl.ds(st, n), :], x_scr.at[pl.ds(st, n), :], sem.at[SX + t])

        def out_copy(t):
            st, n = tile_rows(t)
            return pltpu.make_async_copy(out_scr.at[pl.ds(st, n), :], out_hbm.at[pl.ds(st, n), :], osem.at[t])

        def sec_copy(i):
            s, hf = i // 2, i % 2
            return pltpu.make_async_copy(wqkv_hbm.at[pl.ds(hf * KH, KH), pl.ds(s * D, D)], wqkv_raw.at[i], sem.at[SQ + i])

        def wo_copy():
            return pltpu.make_async_copy(wo_hbm, wo_raw, sem.at[SO])

        def ffn_copies(j):
            return [
                pltpu.make_async_copy(wg_hbm.at[:, pl.ds(j * FC, FC)], wg.at[j], sem.at[SF + 3 * j]),
                pltpu.make_async_copy(wu_hbm.at[:, pl.ds(j * FC, FC)], wu.at[j], sem.at[SF + 3 * j + 1]),
                pltpu.make_async_copy(wd_hbm.at[pl.ds(j * FC, FC), :], wd.at[j], sem.at[SF + 3 * j + 2]),
            ]

        def ln_rows(st, n, dst, dst_r, gate, zero):
            xr = x_scr[pl.ds(st, n), :]
            if gate is not None:
                xi = pltpu.bitcast(xr, I32)
                xi = jnp.concatenate([xi[:, 0:128] | gate, xi[:, 128:]], axis=1)
                xr = pltpu.bitcast(xi, BF)
            x = xr.astype(F32)
            mu = jnp.mean(x, axis=-1, keepdims=True)
            xc = x - mu
            var = jnp.mean(xc * xc, axis=-1, keepdims=True)
            y = (xc * lax.rsqrt(var + 1e-5)).astype(BF)
            dst[dst_r:dst_r + n, :] = y
            if zero is None:
                return None
            pk = pltpu.bitcast(y, I32)
            d = None
            for c in range(8):
                p = pk[:, 128 * c:128 * (c + 1)]
                d = p if d is None else d | p
            return d & zero

        def regroup(j, dst):
            for e in range(16):
                dst[32 * e:32 * (e + 1), 128 * j:128 * (j + 1)] = scru[j, pl.ds(e, 32, stride=PITCH), :]

        def prep_t(i, dst, gates=None):
            for j in range(4):
                for cc in range(8):
                    w = wqkv_raw[i, 128 * j:128 * (j + 1), cc * 128:(cc + 1) * 128]
                    if gates is not None:
                        top = pltpu.bitcast(pltpu.bitcast(w[0:16, :], I32) | gates[j], BF)
                        w = jnp.concatenate([top, w[16:, :]], axis=0)
                    tu = pltpu.bitcast(w.T, U32)
                    for hh in range(4):
                        scru[j, pl.ds(PITCH * (4 * cc + hh), 16), :] = tu[16 * hh:16 * hh + 16, :]
                regroup(j, dst)

        def prep_wo():
            for j in range(8):
                for h in range(H):
                    scru[j, pl.ds(PITCH * h, 16), :] = pltpu.bitcast(wo_raw[32 * h:32 * h + 32, 128 * j:128 * (j + 1)], U32)
                regroup(j, wo_p)

        def ffn_events(g, u, dn, n):
            g0, g3, u0, u2, u3 = g[0:R, 0:128], g[0:R, 384:512], u[0:R, 0:128], u[0:R, 256:384], u[0:R, 384:512]
            dn2, dn4, dn6, dn7 = dn[0:R, 256:384], dn[0:R, 512:640], dn[0:R, 768:896], dn[0:R, 896:1024]
            return {4: [g0, u0, dn2, dn7], 5: [g0, g3, u2, dn2, dn7], 6: [g0, g3, u0, u3, dn2, dn6]}[n]

        def first_tile():
            qkv[1, :, 0:HALO, :] = jnp.zeros((8, HALO, 128), F32)
            with scope('secwait', prof):
                sec_copy(0).wait()
            prep_t(0, wta.at[0])
            with scope('x0wait', prof):
                x_copy(0).wait()
            ln_rows(0, M0, xa, 0, None, None)

            def qkv_body(s, carry):
                with scope('secwait', prof):
                    sec_copy(2 * s + 1).wait()
                r = lax.dot_general(xa[0:M0, 0:KH], wta.bitcast(BF)[s], NT_DIMS, preferred_element_type=F32)
                for c in range(8):
                    qkv[s, c, HALO:HALO + M0, :] = r[:, c * 128:(c + 1) * 128]
                zvec = jnp.full((8, 128), s >> 10, I32)
                prep_t(2 * s + 1, wtb.at[s], [bits(r[0:8, 128 * (j * GM):128 * (j * GM + 1)]) & zvec for j in range(4)])

                @pl.when(s < 2)
                def _():
                    with scope('secwait', prof):
                        sec_copy(2 * s + 2).wait()
                r = lax.dot_general(xa[0:M0, KH:D], wtb.bitcast(BF)[s], NT_DIMS, preferred_element_type=F32)
                for c in range(8):
                    qkv[s, c, HALO:HALO + M0, :] += r[:, c * 128:(c + 1) * 128]
                prep_t(jnp.minimum(2 * s + 2, 5), wta.at[s + 1],
                       [bits(r[0:8, 128 * (j * GM):128 * (j * GM + 1)]) & zvec for j in range(4)])
                return carry
            with scope('f_qkv', prof):
                lax.fori_loop(0, 3, qkv_body, 0)

            for c in range(8):
                qkv[2, c, 0:HALO, :] = jnp.broadcast_to(qkv[2, c, HALO:HALO + 1, :], (HALO, 128))
            acc_scr[0:M0, :] = x_scr[0:M0, :].astype(F32)

            def ffn_body(j, carry):
                with scope('ffnwait', prof):
                    for cp in ffn_copies(j):
                        cp.wait()
                xn = xa[0:M0, :]
                g = jnp.dot(xn, wg[j], preferred_element_type=F32)
                u = jnp.dot(xn, wu[j], preferred_element_type=F32)
                h = (g * u).astype(BF)
                dn = jnp.dot(h, wd[j], preferred_element_type=F32)
                acc_scr[0:M0, :] += dn
                zvec = jnp.full((R, 128), j >> 10, I32)
                evs = [[None, g[0:R, 0:128], g[0:R, 384:512], u[0:R, 0:128], u[0:R, 384:512]],
                       [None, g[0:R, 0:128], g[0:R, 256:384], g[0:R, 384:512], u[0:R, 0:128]],
                       [None, None, g[0:R, 0:128], g[0:R, 384:512], u[0:R, 0:128]]][fev]
                for b in range(BPI):
                    blk = jnp.minimum(j * BPI + b, NB0 - 1)
                    e = evs[b]
                    attn_rows(qkv, o_scr, pl.multiple_of(blk * R, R), True,
                              None if e is None else bits(e) & zvec)
                return carry
            with scope('f_ffn', prof):
                lax.fori_loop(0, NCH, ffn_body, 0)

            wo_copy().wait()
            x_copy(1).wait()
            prep_wo()
            ln_rows(M0, TM, xa, 0, None, None)
            acc = acc_scr[0:M0, :] + jnp.dot(o_scr[0:M0, :], wo_p.bitcast(BF)[...], preferred_element_type=F32)
            out_scr[0:M0, :] = acc.astype(BF)
            out_copy(0).start()
            qkv[1:3, :, 0:HALO, :] = qkv[1:3, :, M0:M0 + HALO, :]

        def steady(t):
            row0, _ = tile_rows(t)
            rown, _ = tile_rows(jnp.minimum(t + 1, NT - 1))

            @pl.when(t + 1 < NT)
            def _():
                x_copy(t + 1).wait()
            zvec = jnp.full((R, 128), t >> 10, I32)

            xn = xa[0:TM, :]
            qkv_ev = []
            for s in range(3):
                r = (lax.dot_general(xn[:, 0:KH], wta.bitcast(BF)[s], NT_DIMS, preferred_element_type=F32)
                     + lax.dot_general(xn[:, KH:D], wtb.bitcast(BF)[s], NT_DIMS, preferred_element_type=F32))
                for c in range(8):
                    qkv[s, c, HALO:HALO + TM, :] = r[:, c * 128:(c + 1) * 128]
                    qkv_ev.append(r[0:R, c * 128:(c + 1) * 128])
            blocks = list(range(0, TM, R))
            nb = len(blocks)
            nuse = last_chunk
            pend = None
            if lnmode == 'free':
                nln = TM // 16
                for i in range(nln):
                    e = qkv_ev[(i * LNSPAN) // nln]
                    ln_rows(rown + 16 * i, 16, xb, 16 * i, bits(e) & zvec, None)
            acc = x_scr[pl.ds(row0, TM), :].astype(F32)
            for j in range(NCH):
                g = jnp.dot(xn, wg[j], preferred_element_type=F32)
                u = jnp.dot(xn, wu[j], preferred_element_type=F32)
                h = (g * u).astype(BF)
                dn = jnp.dot(h, wd[j], preferred_element_type=F32)
                acc = acc + dn
                if j < nuse:
                    lo = j * nb // nuse
                    hi = (j + 1) * nb // nuse
                    evs = ffn_events(g, u, dn, hi - lo)
                    for e, r0 in zip(evs, blocks[lo:hi]):
                        ed = bits(e) & zvec
                        if lnmode == 'free':
                            attn_rows(qkv, o_scr, r0, False, ed)
                        elif r0 % 16 == 0:
                            pend = ln_rows(rown + r0, 16, xb, r0, ed, zvec)
                            attn_rows(qkv, o_scr, r0, False, ed)
                        else:
                            attn_rows(qkv, o_scr, r0, False, ed | pend)
            acc = acc + jnp.dot(o_scr[0:TM, :], wo_p.bitcast(BF)[...], preferred_element_type=F32)
            out_scr[pl.ds(row0, TM), :] = acc.astype(BF)
            out_copy(t).start()
            xa[0:TM, :] = xb[...]
            qkv[1:3, :, 0:HALO, :] = qkv[1:3, :, TM:TM + HALO, :]

        if xfirst:
            x_copy(0).start()
            sec_copy(0).start()
        else:
            sec_copy(0).start()
            x_copy(0).start()
        for i in range(1, 6):
            sec_copy(i).start()
        for j in range(NCH):
            if j == NCH - 1:
                x_copy(1).start()
            for cp in ffn_copies(j):
                cp.start()
        wo_copy().start()
        for t in range(2, NT):
            x_copy(t).start()

        with scope('first', prof):
            first_tile()

        def body(t, carry):
            with scope('steady', prof):
                steady(t)
            return carry
        lax.fori_loop(1, NT, body, 0)

        for t in range(NT):
            out_copy(t).wait()

    @jax.jit
    def run(A_x, A_wqkv, A_wo, B_x, B_w_gate, B_w_up, B_w_down):
        x = A_x.reshape(S, D)
        any_spec = pl.BlockSpec(memory_space=pl.ANY)
        out = pl.pallas_call(
            kernel,
            in_specs=[any_spec] * 6,
            out_specs=any_spec,
            out_shape=jax.ShapeDtypeStruct((S, D), BF),
            scratch_shapes=[
                pltpu.VMEM((S, D), BF), pltpu.VMEM((S, D), BF),
                pltpu.VMEM((TMAX, D), BF), pltpu.VMEM((TM, D), BF),
                pltpu.VMEM((TMAX, D), F32),
                pltpu.VMEM((6, KH, D), BF), pltpu.VMEM((D, D), BF),
                pltpu.VMEM((4, D // 2, KH), U32), pltpu.VMEM((3, D // 2, KH), U32), pltpu.VMEM((D // 2, D), U32),
                pltpu.VMEM((NCH, D, FC), BF), pltpu.VMEM((NCH, D, FC), BF), pltpu.VMEM((NCH, FC, D), BF),
                pltpu.VMEM((3, 8, TMAX + HALO, 128), F32),
                pltpu.VMEM((TMAX, D), BF),
                pltpu.VMEM((8, H * PITCH, 128), U32),
                pltpu.SemaphoreType.DMA((NSEM,)), pltpu.SemaphoreType.DMA((NT,)),
            ],
            compiler_params=pltpu.CompilerParams(vmem_limit_bytes=110 << 20, disable_bounds_checks=nobc),
            name="fused",
        )(x, A_wqkv, A_wo, B_w_gate, B_w_up, B_w_down)
        return out.reshape(1, S, D)

    return run


_run = make_kernel()


@jax.jit
def pallas_parallel_sum__sliding_local_dilated__glu_gated_bilinear__prompt_kernel(
    A_x: jax.Array,
    A_wqkv: jax.Array,
    A_wo: jax.Array,
    B_x: jax.Array,
    B_w_gate: jax.Array,
    B_w_up: jax.Array,
    B_w_down: jax.Array,
):
    return _run(A_x, A_wqkv, A_wo, B_x, B_w_gate, B_w_up, B_w_down)
```

```python
import contextlib
import jax
import jax.numpy as jnp
from jax import lax
import jax.experimental.pallas as pl
import jax.experimental.pallas.tpu as pltpu

S, D, F = 2048, 1024, 3584
H, DH, W, DIL = 32, 32, 8, 2
HALO = 16
NT_DIMS = (((1,), (1,)), ((), ()))
BF = jnp.bfloat16
F32 = jnp.float32
I32 = jnp.int32
U32 = jnp.uint32
R = 8
PITCH = 17
KH = D // 2


def bits(x):
    return lax.bitcast_convert_type(x, I32)


def unbits(x):
    return lax.bitcast_convert_type(x, F32)


def scope(name, on):
    return jax.named_scope(name) if on else contextlib.nullcontext()


def gate_bf16(w, g):
    top = pltpu.bitcast(pltpu.bitcast(w[0:16, 0:128], I32) | g, BF)
    if w.shape[1] > 128:
        top = jnp.concatenate([top, w[0:16, 128:]], axis=1)
    if w.shape[0] > 16:
        top = jnp.concatenate([top, w[16:, :]], axis=0)
    return top


def make_kernel(TM=256, FC=512, last_chunk=5, GM=1, osplit=2, prof=False):
    NT = S // TM
    NCH = F // FC
    SX, SQ, SO, SF = 0, NT, NT + 6, NT + 7
    NSEM = SF + 3 * NCH

    def attn_rows(qkv, o_scr, row0, r0, dep):
        lane = lax.broadcasted_iota(jnp.int32, (R, 128), 1)
        b0 = (lane & 1) == 0
        base = HALO + row0 + r0
        accs = [None] * W
        for c in range(8):
            q = qkv[0, c, pl.ds(base, R), :]
            if c == 0 and dep is not None:
                q = unbits(bits(q) | dep)
            for w in range(W):
                t = q * qkv[1, c, pl.ds(base - DIL * w, R), :]
                accs[w] = t if accs[w] is None else accs[w] + t
        logits = []
        for w in range(W):
            acc = accs[w]
            acc = acc + pltpu.roll(acc, 64, 1)
            acc = acc + jnp.where(b0, pltpu.roll(acc, 127, 1), pltpu.roll(acc, 1, 1))
            lg = acc * (DH ** -0.5)
            if r0 < DIL * w:
                row = lax.broadcasted_iota(jnp.int32, (R, 128), 0) + (row0 + r0)
                lg = jnp.where(row >= DIL * w, lg, -1e9)
            logits.append(lg)
        m = logits[0]
        for w in range(1, W):
            m = jnp.maximum(m, logits[w])
        ps = [jnp.exp(l - m) for l in logits]
        s = ps[0]
        for w in range(1, W):
            s = s + ps[w]
        inv = 1.0 / s
        ps = [p * inv for p in ps]
        for c in range(8):
            o = None
            for w in range(W):
                t = ps[w] * qkv[2, c, pl.ds(base - DIL * w, R), :]
                o = t if o is None else o + t
            o_scr[pl.ds(r0, R), pl.ds(128 * c, 128)] = o.astype(o_scr.dtype)

    def kernel(x_hbm, wqkv_hbm, wo_hbm, wg_hbm, wu_hbm, wd_hbm, out_hbm,
               x_scr, out_scr, xn_all, xa, xb, wqkv_raw, wo_raw, wta, wtb, wo_p, wg, wu, wd,
               qkv, o_scr, scru, sem, osem):
        x_scr, out_scr, xn_all, xa, xb, wqkv_raw, wo_raw, wg, wu, wd, o_scr = [
            r.bitcast(BF) for r in (x_scr, out_scr, xn_all, xa, xb, wqkv_raw, wo_raw, wg, wu, wd, o_scr)]

        def rows(t):
            st = t * TM
            return st if isinstance(st, int) else pl.multiple_of(st, TM)

        def x_copy(t):
            return pltpu.make_async_copy(x_hbm.at[pl.ds(rows(t), TM), :], x_scr.at[pl.ds(rows(t), TM), :], sem.at[SX + t])

        OC = D // osplit

        def out_copy(t, p):
            return pltpu.make_async_copy(out_scr.at[pl.ds(rows(t), TM), pl.ds(p * OC, OC)],
                                         out_hbm.at[pl.ds(rows(t), TM), pl.ds(p * OC, OC)], osem.at[t * osplit + p])

        def sec_copy(i):
            s, hf = i // 2, i % 2
            return pltpu.make_async_copy(wqkv_hbm.at[pl.ds(hf * KH, KH), pl.ds(s * D, D)], wqkv_raw.at[i], sem.at[SQ + i])

        def wo_copy():
            return pltpu.make_async_copy(wo_hbm, wo_raw, sem.at[SO])

        def ffn_copies(j):
            return [
                pltpu.make_async_copy(wg_hbm.at[:, pl.ds(j * FC, FC)], wg.at[j], sem.at[SF + 3 * j]),
                pltpu.make_async_copy(wu_hbm.at[:, pl.ds(j * FC, FC)], wu.at[j], sem.at[SF + 3 * j + 1]),
                pltpu.make_async_copy(wd_hbm.at[pl.ds(j * FC, FC), :], wd.at[j], sem.at[SF + 3 * j + 2]),
            ]

        def ln_rows(st, n, dst, dst_r, gate, zero):
            xr = x_scr[pl.ds(st, n), :]
            if gate is not None:
                xr = gate_bf16(xr, gate)
            x = xr.astype(F32)
            mu = jnp.mean(x, axis=-1, keepdims=True)
            xc = x - mu
            var = jnp.mean(xc * xc, axis=-1, keepdims=True)
            y = (xc * lax.rsqrt(var + 1e-5)).astype(BF)
            dst[dst_r:dst_r + n, :] = y
            if zero is None:
                return None
            pk = pltpu.bitcast(y, I32)
            d = None
            for c in range(8):
                p = pk[:, 128 * c:128 * (c + 1)]
                d = p if d is None else d | p
            return d & zero

        def regroup(j, dst, jd):
            last = None
            for e in range(16):
                last = scru[j, pl.ds(e, 32, stride=PITCH), :]
                dst[32 * e:32 * (e + 1), pl.ds(128 * jd, 128)] = last
            return last

        def prep_t(i, dst, gates=None):
            for j in range(4):
                for cc in range(8):
                    w = wqkv_raw[i, 128 * j:128 * (j + 1), cc * 128:(cc + 1) * 128]
                    if gates is not None:
                        w = gate_bf16(w, gates[j])
                    tu = pltpu.bitcast(w.T, U32)
                    for hh in range(4):
                        scru[j, pl.ds(PITCH * (4 * cc + hh), 16), :] = tu[16 * hh:16 * hh + 16, :]
                regroup(j, dst, j)

        def prep_wo_chunk(j, jd, gate):
            col = pl.multiple_of(jd * 128, 128)
            for h in range(H):
                w = wo_raw[32 * h:32 * h + 32, pl.ds(col, 128)]
                if gate is not None and h == 0:
                    w = gate_bf16(w, gate)
                scru[j, pl.ds(PITCH * h, 16), :] = pltpu.bitcast(w, U32)
            last = None
            for e in range(16):
                last = scru[j, pl.ds(e, 32, stride=PITCH), :]
                wo_p[32 * e:32 * (e + 1), pl.ds(col, 128)] = last
            return last

        def ffn_events(g, u, dn, n):
            g0, g3, u0, u2, u3 = g[0:R, 0:128], g[0:R, 384:512], u[0:R, 0:128], u[0:R, 256:384], u[0:R, 384:512]
            dn2, dn4, dn6, dn7 = dn[0:R, 256:384], dn[0:R, 512:640], dn[0:R, 768:896], dn[0:R, 896:1024]
            return {4: [g0, u0, dn2, dn7], 5: [g0, g3, u2, dn2, dn7], 6: [g0, g3, u0, u3, dn2, dn6],
                    7: [g0, g3, u0, u3, dn2, dn4, dn7]}[n]

        def first_tile():
            qkv[1, :, 0:HALO, :] = jnp.zeros((8, HALO, 128), F32)
            with scope('secwait', prof):
                sec_copy(0).wait()
            prep_t(0, wta.at[0])
            with scope('x0wait', prof):
                x_copy(0).wait()
            ln_rows(0, TM, xa, 0, None, None)
            xn_all[0:TM, :] = xa[...]

            def qkv_body(s, carry):
                with scope('secwait', prof):
                    sec_copy(2 * s + 1).wait()
                r = lax.dot_general(xa[:, 0:KH], wta.bitcast(BF)[s], NT_DIMS, preferred_element_type=F32)
                for c in range(8):
                    qkv[s, c, HALO:HALO + TM, :] = r[:, c * 128:(c + 1) * 128]
                zvec = jnp.full((8, 128), s >> 10, I32)
                prep_t(2 * s + 1, wtb.at[s], [bits(r[0:8, 128 * (j * GM):128 * (j * GM + 1)]) & zvec for j in range(4)])

                @pl.when(s < 2)
                def _():
                    with scope('secwait', prof):
                        sec_copy(2 * s + 2).wait()
                r = lax.dot_general(xa[:, KH:D], wtb.bitcast(BF)[s], NT_DIMS, preferred_element_type=F32)
                for c in range(8):
                    qkv[s, c, HALO:HALO + TM, :] += r[:, c * 128:(c + 1) * 128]
                prep_t(jnp.minimum(2 * s + 2, 5), wta.at[s + 1],
                       [bits(r[0:8, 128 * (j * GM):128 * (j * GM + 1)]) & zvec for j in range(4)])
                return carry
            with scope('f_qkv', prof):
                lax.fori_loop(0, 3, qkv_body, 0)

            for c in range(8):
                qkv[2, c, 0:HALO, :] = jnp.broadcast_to(qkv[2, c, HALO:HALO + 1, :], (HALO, 128))
            x_copy(1).wait()
            wo_copy().wait()
            ln_rows(TM, TM, xa, 0, None, None)
            xn_all[TM:2 * TM, :] = xa[...]

        def phase_a(t):
            row0 = rows(t)
            tn = jnp.minimum(t + 1, NT - 1)
            rown = rows(tn)

            @pl.when(t + 1 < NT)
            def _():
                x_copy(t + 1).wait()
            zvec = jnp.full((8, 128), t >> 10, I32)
            xn = xa[...]
            tok = None
            for s in range(3):
                lo, hi = xn[:, 0:KH], xn[:, KH:D]
                if s == 2:
                    lo = gate_bf16(lo, tok)
                rl = lax.dot_general(lo, wta.bitcast(BF)[s], NT_DIMS, preferred_element_type=F32)
                r = rl + lax.dot_general(hi, wtb.bitcast(BF)[s], NT_DIMS, preferred_element_type=F32)
                for c in range(8):
                    qkv[s, c, pl.ds(HALO + row0, TM), :] = r[:, c * 128:(c + 1) * 128]
                evs = ([bits(rl[0:8, 128 * i:128 * (i + 1)]) & zvec for i in range(8)]
                       + [bits(r[0:8, 128 * i:128 * (i + 1)]) & zvec for i in range(8)])
                if s == 0:
                    for i in range(16):
                        d = ln_rows(rown + 16 * i, 16, xb, 16 * i, evs[i], zvec)
                        tok = d if tok is None else tok | d
                if s == 1:
                    for k in range(2):
                        jd = jnp.minimum(2 * (t - 1) + k, 7)
                        last = prep_wo_chunk(k, jd, evs[3 * k])
                        tok = tok | (lax.bitcast_convert_type(last[0:8, :], I32) & zvec)
            xa[...] = xb[...]
            xn_all[pl.ds(rown, TM), :] = xb[...]

        def phase_b(t):
            row0 = rows(t)
            zvec = jnp.full((R, 128), t >> 10, I32)
            xn = xn_all[pl.ds(row0, TM), :]
            blocks = list(range(0, TM, R))
            nb = len(blocks)
            nuse = last_chunk
            acc = x_scr[pl.ds(row0, TM), :].astype(F32)
            for j in range(NCH):
                g = jnp.dot(xn, wg[j], preferred_element_type=F32)
                u = jnp.dot(xn, wu[j], preferred_element_type=F32)
                h = (g * u).astype(BF)
                dn = jnp.dot(h, wd[j], preferred_element_type=F32)
                acc = acc + dn
                if j < nuse:
                    lo = j * nb // nuse
                    hi = (j + 1) * nb // nuse
                    evs = ffn_events(g, u, dn, hi - lo)
                    for e, r0 in zip(evs, blocks[lo:hi]):
                        attn_rows(qkv, o_scr, row0, r0, bits(e) & zvec)
            acc = acc + jnp.dot(o_scr[...], wo_p.bitcast(BF)[...], preferred_element_type=F32)
            for p in range(osplit):
                out_scr[pl.ds(row0, TM), p * OC:(p + 1) * OC] = acc[:, p * OC:(p + 1) * OC].astype(BF)
                out_copy(t, p).start()

        sec_copy(0).start()
        x_copy(0).start()
        for i in range(1, 6):
            sec_copy(i).start()
        x_copy(1).start()
        wo_copy().start()
        x_copy(2).start()
        for j in range(NCH):
            for cp in ffn_copies(j):
                cp.start()
            if j + 3 < NT:
                x_copy(j + 3).start()

        with scope('first', prof):
            first_tile()

        def body_a(t, carry):
            with scope('phase_a', prof):
                phase_a(t)
            return carry
        lax.fori_loop(1, NT, body_a, 0)

        for j in range(NCH):
            for cp in ffn_copies(j):
                cp.wait()

        def body_b(t, carry):
            with scope('phase_b', prof):
                phase_b(t)
            return carry
        lax.fori_loop(0, NT, body_b, 0)

        for t in range(NT):
            for p in range(osplit):
                out_copy(t, p).wait()

    @jax.jit
    def run(A_x, A_wqkv, A_wo, B_x, B_w_gate, B_w_up, B_w_down):
        x = A_x.reshape(S, D)
        any_spec = pl.BlockSpec(memory_space=pl.ANY)
        out = pl.pallas_call(
            kernel,
            in_specs=[any_spec] * 6,
            out_specs=any_spec,
            out_shape=jax.ShapeDtypeStruct((S, D), BF),
            scratch_shapes=[
                pltpu.VMEM((S // 2, D), U32), pltpu.VMEM((S // 2, D), U32), pltpu.VMEM((S // 2, D), U32),
                pltpu.VMEM((TM // 2, D), U32), pltpu.VMEM((TM // 2, D), U32),
                pltpu.VMEM((6, KH // 2, D), U32), pltpu.VMEM((D // 2, D), U32),
                pltpu.VMEM((4, D // 2, KH), U32), pltpu.VMEM((3, D // 2, KH), U32), pltpu.VMEM((D // 2, D), U32),
                pltpu.VMEM((NCH, D // 2, FC), U32), pltpu.VMEM((NCH, D // 2, FC), U32), pltpu.VMEM((NCH, FC // 2, D), U32),
                pltpu.VMEM((3, 8, S + HALO, 128), F32),
                pltpu.VMEM((TM // 2, D), U32),
                pltpu.VMEM((4, H * PITCH, 128), U32),
                pltpu.SemaphoreType.DMA((NSEM,)), pltpu.SemaphoreType.DMA((NT * osplit,)),
            ],
            compiler_params=pltpu.CompilerParams(vmem_limit_bytes=120 << 20),
            name="fused",
        )(x, A_wqkv, A_wo, B_w_gate, B_w_up, B_w_down)
        return out.reshape(1, S, D)

    return run


_run = make_kernel()


@jax.jit
def pallas_parallel_sum__sliding_local_dilated__glu_gated_bilinear__prompt_kernel(
    A_x: jax.Array,
    A_wqkv: jax.Array,
    A_wo: jax.Array,
    B_x: jax.Array,
    B_w_gate: jax.Array,
    B_w_up: jax.Array,
    B_w_down: jax.Array,
):
    return _run(A_x, A_wqkv, A_wo, B_x, B_w_gate, B_w_up, B_w_down)
```

```python
import contextlib
import jax
import jax.numpy as jnp
from jax import lax
import jax.experimental.pallas as pl
import jax.experimental.pallas.tpu as pltpu

S, D, F = 2048, 1024, 3584
H, DH, W, DIL = 32, 32, 8, 2
HALO = 16
NT_DIMS = (((1,), (1,)), ((), ()))
BF = jnp.bfloat16
F32 = jnp.float32
I32 = jnp.int32
U32 = jnp.uint32
R = 8
PITCH = 17
KH = D // 2


def bits(x):
    return lax.bitcast_convert_type(x, I32)


def unbits(x):
    return lax.bitcast_convert_type(x, F32)


def scope(name, on):
    return jax.named_scope(name) if on else contextlib.nullcontext()


def gate_bf16(w, g):
    top = pltpu.bitcast(pltpu.bitcast(w[0:16, 0:128], I32) | g, BF)
    if w.shape[1] > 128:
        top = jnp.concatenate([top, w[0:16, 128:]], axis=1)
    if w.shape[0] > 16:
        top = jnp.concatenate([top, w[16:, :]], axis=0)
    return top


def make_kernel(TM=256, FC=512, last_chunk=5, GM=1, osplit=2, lnv=3, achain=1, pvchain=1, qkchain=0, prof=False):
    NT = S // TM
    NCH = F // FC
    SX, SQ, SO, SF = 0, NT, NT + 6, NT + 7
    NSEM = SF + 3 * NCH

    def attn_rows(qkv, o_scr, row0, r0, dep, zvec):
        lane = lax.broadcasted_iota(jnp.int32, (R, 128), 1)
        b0 = (lane & 1) == 0
        base = HALO + row0 + r0
        accs = [None] * W
        for c in range(8):
            q = qkv[0, c, pl.ds(base, R), :]
            if c == 0 and dep is not None:
                q = unbits(bits(q) | dep)
            if qkchain and c > 0 and c % qkchain == 0:
                q = unbits(bits(q) | (bits(accs[W - 1]) & zvec))
            for w in range(W):
                t = q * qkv[1, c, pl.ds(base - DIL * w, R), :]
                accs[w] = t if accs[w] is None else accs[w] + t
        logits = []
        for w in range(W):
            acc = accs[w]
            acc = acc + pltpu.roll(acc, 64, 1)
            acc = acc + jnp.where(b0, pltpu.roll(acc, 127, 1), pltpu.roll(acc, 1, 1))
            lg = acc * (DH ** -0.5)
            if r0 < DIL * w:
                row = lax.broadcasted_iota(jnp.int32, (R, 128), 0) + (row0 + r0)
                lg = jnp.where(row >= DIL * w, lg, -1e9)
            logits.append(lg)
        m = logits[0]
        for w in range(1, W):
            m = jnp.maximum(m, logits[w])
        ps = [jnp.exp(l - m) for l in logits]
        s = ps[0]
        for w in range(1, W):
            s = s + ps[w]
        inv = 1.0 / s
        ps = [p * inv for p in ps]
        o = None
        for c in range(8):
            po = o if c > 0 else None
            o = None
            for w in range(W):
                p = ps[w]
                if pvchain and c > 0 and c % pvchain == 0:
                    p = unbits(bits(p) | (bits(po) & zvec)) if w == 0 else p
                t = p * qkv[2, c, pl.ds(base - DIL * w, R), :]
                o = t if o is None else o + t
            o_scr[pl.ds(r0, R), pl.ds(128 * c, 128)] = o.astype(o_scr.dtype)
        return o

    def kernel(x_hbm, wqkv_hbm, wo_hbm, wg_hbm, wu_hbm, wd_hbm, out_hbm,
               x_scr, out_scr, xn_all, xa, xb, wqkv_raw, wo_raw, wta, wtb, wo_p, wg, wu, wd,
               qkv, o_scr, scru, sem, osem):
        x_scr, out_scr, xn_all, xa, xb, wqkv_raw, wo_raw, wg, wu, wd, o_scr = [
            r.bitcast(BF) for r in (x_scr, out_scr, xn_all, xa, xb, wqkv_raw, wo_raw, wg, wu, wd, o_scr)]

        def rows(t):
            st = t * TM
            return st if isinstance(st, int) else pl.multiple_of(st, TM)

        def x_copy(t):
            return pltpu.make_async_copy(x_hbm.at[pl.ds(rows(t), TM), :], x_scr.at[pl.ds(rows(t), TM), :], sem.at[SX + t])

        OC = D // osplit

        def out_copy(t, p):
            return pltpu.make_async_copy(out_scr.at[pl.ds(rows(t), TM), pl.ds(p * OC, OC)],
                                         out_hbm.at[pl.ds(rows(t), TM), pl.ds(p * OC, OC)], osem.at[t * osplit + p])

        def sec_copy(i):
            s, hf = i // 2, i % 2
            return pltpu.make_async_copy(wqkv_hbm.at[pl.ds(hf * KH, KH), pl.ds(s * D, D)], wqkv_raw.at[i], sem.at[SQ + i])

        def wo_copy():
            return pltpu.make_async_copy(wo_hbm, wo_raw, sem.at[SO])

        def ffn_copies(j):
            return [
                pltpu.make_async_copy(wg_hbm.at[:, pl.ds(j * FC, FC)], wg.at[j], sem.at[SF + 3 * j]),
                pltpu.make_async_copy(wu_hbm.at[:, pl.ds(j * FC, FC)], wu.at[j], sem.at[SF + 3 * j + 1]),
                pltpu.make_async_copy(wd_hbm.at[pl.ds(j * FC, FC), :], wd.at[j], sem.at[SF + 3 * j + 2]),
            ]

        def ln_rows(st, n, dst, dst_r, gate, zero):
            xr = x_scr[pl.ds(st, n), :]
            if gate is not None:
                xr = gate_bf16(xr, gate)
            x = xr.astype(F32)
            mu = jnp.mean(x, axis=-1, keepdims=True)
            xc = x - mu
            var = jnp.mean(xc * xc, axis=-1, keepdims=True)
            y = (xc * lax.rsqrt(var + 1e-5)).astype(BF)
            dst[dst_r:dst_r + n, :] = y
            if zero is None:
                return None
            pk = pltpu.bitcast(y, I32)
            d = None
            for c in range(8):
                p = pk[:, 128 * c:128 * (c + 1)]
                d = p if d is None else d | p
            return d & zero

        def regroup(j, dst, jd):
            last = None
            for e in range(16):
                last = scru[j, pl.ds(e, 32, stride=PITCH), :]
                dst[32 * e:32 * (e + 1), pl.ds(128 * jd, 128)] = last
            return last

        def prep_t(i, dst, gates=None):
            for j in range(4):
                for cc in range(8):
                    w = wqkv_raw[i, 128 * j:128 * (j + 1), cc * 128:(cc + 1) * 128]
                    if gates is not None:
                        w = gate_bf16(w, gates[j])
                    tu = pltpu.bitcast(w.T, U32)
                    for hh in range(4):
                        scru[j, pl.ds(PITCH * (4 * cc + hh), 16), :] = tu[16 * hh:16 * hh + 16, :]
                regroup(j, dst, j)

        def prep_wo_chunk(j, jd, gate):
            col = pl.multiple_of(jd * 128, 128)
            for h in range(H):
                w = wo_raw[32 * h:32 * h + 32, pl.ds(col, 128)]
                if gate is not None and h == 0:
                    w = gate_bf16(w, gate)
                scru[j, pl.ds(PITCH * h, 16), :] = pltpu.bitcast(w, U32)
            last = None
            for e in range(16):
                last = scru[j, pl.ds(e, 32, stride=PITCH), :]
                wo_p[32 * e:32 * (e + 1), pl.ds(col, 128)] = last
            return last

        def ffn_events(g, u, dn, n):
            g0, g3, u0, u2, u3 = g[0:R, 0:128], g[0:R, 384:512], u[0:R, 0:128], u[0:R, 256:384], u[0:R, 384:512]
            dn2, dn4, dn6, dn7 = dn[0:R, 256:384], dn[0:R, 512:640], dn[0:R, 768:896], dn[0:R, 896:1024]
            return {4: [g0, u0, dn2, dn7], 5: [g0, g3, u2, dn2, dn7], 6: [g0, g3, u0, u3, dn2, dn6],
                    7: [g0, g3, u0, u3, dn2, dn4, dn7]}[n]

        def first_tile():
            qkv[1, :, 0:HALO, :] = jnp.zeros((8, HALO, 128), F32)
            with scope('secwait', prof):
                sec_copy(0).wait()
            prep_t(0, wta.at[0])
            with scope('x0wait', prof):
                x_copy(0).wait()
            ln_rows(0, TM, xa, 0, None, None)
            xn_all[0:TM, :] = xa[...]

            def qkv_body(s, carry):
                with scope('secwait', prof):
                    sec_copy(2 * s + 1).wait()
                r = lax.dot_general(xa[:, 0:KH], wta.bitcast(BF)[s], NT_DIMS, preferred_element_type=F32)
                for c in range(8):
                    qkv[s, c, HALO:HALO + TM, :] = r[:, c * 128:(c + 1) * 128]
                zvec = jnp.full((8, 128), s >> 10, I32)
                prep_t(2 * s + 1, wtb.at[s], [bits(r[0:8, 128 * (j * GM):128 * (j * GM + 1)]) & zvec for j in range(4)])

                @pl.when(s < 2)
                def _():
                    with scope('secwait', prof):
                        sec_copy(2 * s + 2).wait()
                r = lax.dot_general(xa[:, KH:D], wtb.bitcast(BF)[s], NT_DIMS, preferred_element_type=F32)
                for c in range(8):
                    qkv[s, c, HALO:HALO + TM, :] += r[:, c * 128:(c + 1) * 128]
                prep_t(jnp.minimum(2 * s + 2, 5), wta.at[s + 1],
                       [bits(r[0:8, 128 * (j * GM):128 * (j * GM + 1)]) & zvec for j in range(4)])
                return carry
            with scope('f_qkv', prof):
                lax.fori_loop(0, 3, qkv_body, 0)

            for c in range(8):
                qkv[2, c, 0:HALO, :] = jnp.broadcast_to(qkv[2, c, HALO:HALO + 1, :], (HALO, 128))
            x_copy(1).wait()
            wo_copy().wait()
            ln_rows(TM, TM, xa, 0, None, None)
            xn_all[TM:2 * TM, :] = xa[...]

        def phase_a(t):
            row0 = rows(t)
            tn = jnp.minimum(t + 1, NT - 1)
            rown = rows(tn)

            @pl.when(t + 1 < NT)
            def _():
                x_copy(t + 1).wait()
            zvec = jnp.full((8, 128), t >> 10, I32)
            xn = xa[...]
            toks = {}
            prevs = {}

            def add_tok(key, d):
                toks[key] = d if key not in toks else toks[key] | d

            for s in range(3):
                lo, hi = xn[:, 0:KH], xn[:, KH:D]
                if (s, 0) in toks:
                    lo = gate_bf16(lo, toks[(s, 0)])
                if (s, 1) in toks:
                    hi = gate_bf16(hi, toks[(s, 1)])
                rl = lax.dot_general(lo, wta.bitcast(BF)[s], NT_DIMS, preferred_element_type=F32)
                r = rl + lax.dot_general(hi, wtb.bitcast(BF)[s], NT_DIMS, preferred_element_type=F32)
                for c in range(8):
                    qkv[s, c, pl.ds(HALO + row0, TM), :] = r[:, c * 128:(c + 1) * 128]
                evs = ([bits(rl[0:8, 128 * i:128 * (i + 1)]) & zvec for i in range(8)]
                       + [bits(r[0:8, 128 * i:128 * (i + 1)]) & zvec for i in range(8)])
                if lnv == 0:
                    plan = [(0, i, (2, 0)) for i in range(16)]
                    woplan = [(1, 0, (2, 0)), (1, 3, (2, 0))]
                elif lnv == 1:
                    plan = [(0, 2 * i, (1, 1)) for i in range(8)] + [(1, 2 * i, (2, 1)) for i in range(8)]
                    woplan = [(0, 1, (1, 1)), (1, 1, (2, 1))]
                elif lnv == 2:
                    plan = ([(0, i, (1, 0)) for i in range(0, 6)] + [(0, i, (1, 1)) for i in range(8, 13)]
                            + [(1, i, (2, 0)) for i in range(0, 5)])
                    woplan = [(1, 8, (2, 1)), (1, 10, (2, 1))]
                elif lnv == 3:
                    plan = [(0, i, (2, 0)) for i in range(16)]
                    woplan = [(1, 0, (2, 0)), (1, 3, (2, 0))]
                elif lnv == 4:
                    plan = [(0, i, (2, 1)) for i in range(0, 16, 2)] + [(0, 15, (2, 1))] + [(1, i, (2, 1)) for i in range(0, 7)]
                    woplan = [(1, 8, (2, 1)), (1, 11, (2, 1))]
                elif lnv == 5:
                    plan = [(0, i, (2, 1)) for i in range(16)]
                    woplan = [(1, 0, (2, 1)), (1, 4, (2, 1))]
                if s == 0:
                    prevs['p'] = None
                prev = prevs['p']
                for i, (es, ei, cons) in enumerate(plan):
                    if es == s:
                        g = evs[ei]
                        if lnv >= 3 and prev is not None:
                            g = g | prev
                        d = ln_rows(rown + 16 * i, 16, xb, 16 * i, g, zvec)
                        prev = d
                        prevs['p'] = d
                        add_tok(cons, d)
                for k, (es, ei, cons) in enumerate(woplan):
                    if es == s:
                        jd = jnp.minimum(2 * (t - 1) + k, 7)
                        last = prep_wo_chunk(k, jd, evs[ei])
                        add_tok(cons, lax.bitcast_convert_type(last[0:8, :], I32) & zvec)
            xa[...] = xb[...]
            xn_all[pl.ds(rown, TM), :] = xb[...]

        def phase_b(t):
            row0 = rows(t)
            zvec = jnp.full((R, 128), t >> 10, I32)
            xn = xn_all[pl.ds(row0, TM), :]
            blocks = list(range(0, TM, R))
            nb = len(blocks)
            nuse = last_chunk
            acc = x_scr[pl.ds(row0, TM), :].astype(F32)
            prev_o = None
            for j in range(NCH):
                g = jnp.dot(xn, wg[j], preferred_element_type=F32)
                u = jnp.dot(xn, wu[j], preferred_element_type=F32)
                h = (g * u).astype(BF)
                dn = jnp.dot(h, wd[j], preferred_element_type=F32)
                acc = acc + dn
                if j < nuse:
                    lo = j * nb // nuse
                    hi = (j + 1) * nb // nuse
                    evs = ffn_events(g, u, dn, hi - lo)
                    for e, r0 in zip(evs, blocks[lo:hi]):
                        g = bits(e) & zvec
                        if achain and prev_o is not None:
                            g = g | prev_o
                        o = attn_rows(qkv, o_scr, row0, r0, g, zvec)
                        prev_o = bits(o) & zvec
            acc = acc + jnp.dot(o_scr[...], wo_p.bitcast(BF)[...], preferred_element_type=F32)
            for p in range(osplit):
                out_scr[pl.ds(row0, TM), p * OC:(p + 1) * OC] = acc[:, p * OC:(p + 1) * OC].astype(BF)
                out_copy(t, p).start()

        sec_copy(0).start()
        x_copy(0).start()
        for i in range(1, 6):
            sec_copy(i).start()
        x_copy(1).start()
        wo_copy().start()
        x_copy(2).start()
        for j in range(NCH):
            for cp in ffn_copies(j):
                cp.start()
            if j + 3 < NT:
                x_copy(j + 3).start()

        with scope('first', prof):
            first_tile()

        def body_a(t, carry):
            with scope('phase_a', prof):
                phase_a(t)
            return carry
        lax.fori_loop(1, NT, body_a, 0)

        for j in range(NCH):
            for cp in ffn_copies(j):
                cp.wait()

        def body_b(t, carry):
            with scope('phase_b', prof):
                phase_b(t)
            return carry
        lax.fori_loop(0, NT, body_b, 0)

        for t in range(NT):
            for p in range(osplit):
                out_copy(t, p).wait()

    @jax.jit
    def run(A_x, A_wqkv, A_wo, B_x, B_w_gate, B_w_up, B_w_down):
        x = A_x.reshape(S, D)
        any_spec = pl.BlockSpec(memory_space=pl.ANY)
        out = pl.pallas_call(
            kernel,
            in_specs=[any_spec] * 6,
            out_specs=any_spec,
            out_shape=jax.ShapeDtypeStruct((S, D), BF),
            scratch_shapes=[
                pltpu.VMEM((S // 2, D), U32), pltpu.VMEM((S // 2, D), U32), pltpu.VMEM((S // 2, D), U32),
                pltpu.VMEM((TM // 2, D), U32), pltpu.VMEM((TM // 2, D), U32),
                pltpu.VMEM((6, KH // 2, D), U32), pltpu.VMEM((D // 2, D), U32),
                pltpu.VMEM((4, D // 2, KH), U32), pltpu.VMEM((3, D // 2, KH), U32), pltpu.VMEM((D // 2, D), U32),
                pltpu.VMEM((NCH, D // 2, FC), U32), pltpu.VMEM((NCH, D // 2, FC), U32), pltpu.VMEM((NCH, FC // 2, D), U32),
                pltpu.VMEM((3, 8, S + HALO, 128), F32),
                pltpu.VMEM((TM // 2, D), U32),
                pltpu.VMEM((4, H * PITCH + 32, 128), U32),
                pltpu.SemaphoreType.DMA((NSEM,)), pltpu.SemaphoreType.DMA((NT * osplit,)),
            ],
            compiler_params=pltpu.CompilerParams(vmem_limit_bytes=120 << 20),
            name="fused",
        )(x, A_wqkv, A_wo, B_w_gate, B_w_up, B_w_down)
        return out.reshape(1, S, D)

    return run


_run = make_kernel()


@jax.jit
def pallas_parallel_sum__sliding_local_dilated__glu_gated_bilinear__prompt_kernel(
    A_x: jax.Array,
    A_wqkv: jax.Array,
    A_wo: jax.Array,
    B_x: jax.Array,
    B_w_gate: jax.Array,
    B_w_up: jax.Array,
    B_w_down: jax.Array,
):
    return _run(A_x, A_wqkv, A_wo, B_x, B_w_gate, B_w_up, B_w_down)
```

```python
import jax
import jax.numpy as jnp
from jax import lax
import jax.experimental.pallas as pl
import jax.experimental.pallas.tpu as pltpu

S, D, F = 2048, 1024, 3584
H, DH, W, DIL = 32, 32, 8, 2
EPS = 1e-5
HALO = 16
TM = 256
NT = S // TM
FC = 512
NCH = F // FC
KH = D // 2
R = 8
PITCH = 17
ATTN_CHUNKS = 5
OSPLIT = 2
OC = D // OSPLIT

BF = jnp.bfloat16
F32 = jnp.float32
I32 = jnp.int32
U32 = jnp.uint32
NT_DIMS = (((1,), (1,)), ((), ()))

SEM_X, SEM_QKV, SEM_WO, SEM_FFN = 0, NT, NT + 6, NT + 7
NSEM = SEM_FFN + 3 * NCH


def _bits(x):
    return lax.bitcast_convert_type(x, I32)


def _unbits(x):
    return lax.bitcast_convert_type(x, F32)


def _gate_bf16(w, tok):
    top = pltpu.bitcast(pltpu.bitcast(w[0:16, 0:128], I32) | tok, BF)
    if w.shape[1] > 128:
        top = jnp.concatenate([top, w[0:16, 128:]], axis=1)
    if w.shape[0] > 16:
        top = jnp.concatenate([top, w[16:, :]], axis=0)
    return top


def _dot_nt(a, b):
    return lax.dot_general(a, b, NT_DIMS, preferred_element_type=F32)


def _dot(a, b):
    return jnp.dot(a, b, preferred_element_type=F32)


def _attn_block(qkv, o_scr, row0, r0, tok, zero):
    lane = lax.broadcasted_iota(I32, (R, 128), 1)
    even = (lane & 1) == 0
    base = HALO + row0 + r0
    accs = [None] * W
    for c in range(8):
        q = qkv[0, c, pl.ds(base, R), :]
        if c == 0:
            q = _unbits(_bits(q) | tok)
        for w in range(W):
            t = q * qkv[1, c, pl.ds(base - DIL * w, R), :]
            accs[w] = t if accs[w] is None else accs[w] + t
    logits = []
    for w in range(W):
        acc = accs[w]
        acc = acc + pltpu.roll(acc, 64, 1)
        acc = acc + jnp.where(even, pltpu.roll(acc, 127, 1), pltpu.roll(acc, 1, 1))
        lg = acc * (DH ** -0.5)
        if r0 < DIL * w:
            row = lax.broadcasted_iota(I32, (R, 128), 0) + (row0 + r0)
            lg = jnp.where(row >= DIL * w, lg, -1e9)
        logits.append(lg)
    m = logits[0]
    for w in range(1, W):
        m = jnp.maximum(m, logits[w])
    ps = [jnp.exp(l - m) for l in logits]
    den = ps[0]
    for w in range(1, W):
        den = den + ps[w]
    inv = 1.0 / den
    ps = [p * inv for p in ps]
    o = None
    for c in range(8):
        p0 = ps[0] if o is None else _unbits(_bits(ps[0]) | (_bits(o) & zero))
        o = p0 * qkv[2, c, pl.ds(base, R), :]
        for w in range(1, W):
            o = o + ps[w] * qkv[2, c, pl.ds(base - DIL * w, R), :]
        o_scr[pl.ds(r0, R), pl.ds(128 * c, 128)] = o.astype(BF)
    return _bits(o) & zero


def _kernel(x_hbm, wqkv_hbm, wo_hbm, wg_hbm, wu_hbm, wd_hbm, out_hbm,
            x_scr, out_scr, xn_all, xa, xb, wqkv_raw, wo_raw, wg, wu, wd, o_scr,
            wta, wtb, wo_p, qkv, stage, sem, osem):
    x_scr, out_scr, xn_all, xa, xb, wqkv_raw, wo_raw, wg, wu, wd, o_scr = [
        r.bitcast(BF) for r in (x_scr, out_scr, xn_all, xa, xb, wqkv_raw, wo_raw, wg, wu, wd, o_scr)]
    wta_bf, wtb_bf, wo_bf = wta.bitcast(BF), wtb.bitcast(BF), wo_p.bitcast(BF)

    def rows(t):
        return t * TM if isinstance(t, int) else pl.multiple_of(t * TM, TM)

    def x_copy(t):
        return pltpu.make_async_copy(x_hbm.at[pl.ds(rows(t), TM), :], x_scr.at[pl.ds(rows(t), TM), :],
                                     sem.at[SEM_X + t])

    def out_copy(t, p):
        return pltpu.make_async_copy(out_scr.at[pl.ds(rows(t), TM), pl.ds(p * OC, OC)],
                                     out_hbm.at[pl.ds(rows(t), TM), pl.ds(p * OC, OC)], osem.at[t * OSPLIT + p])

    def qkv_copy(i):
        return pltpu.make_async_copy(wqkv_hbm.at[pl.ds((i % 2) * KH, KH), pl.ds((i // 2) * D, D)],
                                     wqkv_raw.at[i], sem.at[SEM_QKV + i])

    def wo_copy():
        return pltpu.make_async_copy(wo_hbm, wo_raw, sem.at[SEM_WO])

    def ffn_copies(j):
        return [
            pltpu.make_async_copy(wg_hbm.at[:, pl.ds(j * FC, FC)], wg.at[j], sem.at[SEM_FFN + 3 * j]),
            pltpu.make_async_copy(wu_hbm.at[:, pl.ds(j * FC, FC)], wu.at[j], sem.at[SEM_FFN + 3 * j + 1]),
            pltpu.make_async_copy(wd_hbm.at[pl.ds(j * FC, FC), :], wd.at[j], sem.at[SEM_FFN + 3 * j + 2]),
        ]

    def layernorm(src, n, dst, dst_row, tok=None, zero=None):
        xr = x_scr[pl.ds(src, n), :]
        if tok is not None:
            xr = _gate_bf16(xr, tok)
        x = xr.astype(F32)
        mu = jnp.mean(x, axis=-1, keepdims=True)
        xc = x - mu
        var = jnp.mean(xc * xc, axis=-1, keepdims=True)
        y = (xc * lax.rsqrt(var + EPS)).astype(BF)
        dst[dst_row:dst_row + n, :] = y
        if zero is None:
            return None
        pk = pltpu.bitcast(y, I32)
        d = pk[:, 0:128]
        for c in range(1, 8):
            d = d | pk[:, 128 * c:128 * (c + 1)]
        return d & zero

    def regroup(j, dst, col):
        v = None
        for e in range(16):
            v = stage[j, pl.ds(e, 32, stride=PITCH), :]
            dst[32 * e:32 * (e + 1), pl.ds(col, 128)] = v
        return v

    def prep_qkv(i, dst, toks=None):
        for j in range(4):
            for cc in range(8):
                w = wqkv_raw[i, 128 * j:128 * (j + 1), 128 * cc:128 * (cc + 1)]
                if toks is not None:
                    w = _gate_bf16(w, toks[j])
                tu = pltpu.bitcast(w.T, U32)
                for hh in range(4):
                    stage[j, pl.ds(PITCH * (4 * cc + hh), 16), :] = tu[16 * hh:16 * hh + 16, :]
            regroup(j, dst, 128 * j)

    def prep_wo(j, jd, tok, zero):
        col = pl.multiple_of(jd * 128, 128)
        for h in range(H):
            w = wo_raw[32 * h:32 * h + 32, pl.ds(col, 128)]
            if h == 0:
                w = _gate_bf16(w, tok)
            stage[j, pl.ds(PITCH * h, 16), :] = pltpu.bitcast(w, U32)
        v = regroup(j, wo_p, col)
        return lax.bitcast_convert_type(v[0:8, :], I32) & zero

    def tile_tokens(r, n, zero):
        return [_bits(r[0:8, 128 * i:128 * (i + 1)]) & zero for i in range(n)]

    def first_tile():
        qkv[1, :, 0:HALO, :] = jnp.zeros((8, HALO, 128), F32)
        qkv_copy(0).wait()
        prep_qkv(0, wta.at[0])
        x_copy(0).wait()
        layernorm(0, TM, xa, 0)
        xn_all[0:TM, :] = xa[...]

        def section(s, carry):
            zero = jnp.full((8, 128), s >> 10, I32)
            qkv_copy(2 * s + 1).wait()
            r = _dot_nt(xa[:, 0:KH], wta_bf[s])
            for c in range(8):
                qkv[s, c, HALO:HALO + TM, :] = r[:, 128 * c:128 * (c + 1)]
            prep_qkv(2 * s + 1, wtb.at[s], tile_tokens(r, 4, zero))

            @pl.when(s < 2)
            def _():
                qkv_copy(2 * s + 2).wait()
            r = _dot_nt(xa[:, KH:D], wtb_bf[s])
            for c in range(8):
                qkv[s, c, HALO:HALO + TM, :] += r[:, 128 * c:128 * (c + 1)]
            prep_qkv(jnp.minimum(2 * s + 2, 5), wta.at[s + 1], tile_tokens(r, 4, zero))
            return carry
        lax.fori_loop(0, 3, section, 0)

        for c in range(8):
            qkv[2, c, 0:HALO, :] = jnp.broadcast_to(qkv[2, c, HALO:HALO + 1, :], (HALO, 128))
        x_copy(1).wait()
        wo_copy().wait()
        layernorm(TM, TM, xa, 0)
        xn_all[TM:2 * TM, :] = xa[...]

    def phase_a(t, carry):
        row0 = rows(t)
        rown = rows(jnp.minimum(t + 1, NT - 1))

        @pl.when(t + 1 < NT)
        def _():
            x_copy(t + 1).wait()
        zero = jnp.full((8, 128), t >> 10, I32)
        xn = xa[...]
        done = None
        for s in range(3):
            lo, hi = xn[:, 0:KH], xn[:, KH:D]
            if s == 2:
                lo = _gate_bf16(lo, done)
            rl = _dot_nt(lo, wta_bf[s])
            r = rl + _dot_nt(hi, wtb_bf[s])
            for c in range(8):
                qkv[s, c, pl.ds(HALO + row0, TM), :] = r[:, 128 * c:128 * (c + 1)]
            toks = tile_tokens(rl, 8, zero) + tile_tokens(r, 8, zero)
            if s == 0:
                prev = None
                for i in range(TM // 16):
                    g = toks[i] if prev is None else toks[i] | prev
                    prev = layernorm(rown + 16 * i, 16, xb, 16 * i, g, zero)
                    done = prev if done is None else done | prev
            if s == 1:
                for k in range(2):
                    done = done | prep_wo(k, jnp.minimum(2 * (t - 1) + k, 7), toks[3 * k], zero)
        xa[...] = xb[...]
        xn_all[pl.ds(rown, TM), :] = xb[...]
        return carry

    def phase_b(t, carry):
        row0 = rows(t)
        zero = jnp.full((R, 128), t >> 10, I32)
        xn = xn_all[pl.ds(row0, TM), :]
        blocks = list(range(0, TM, R))
        nb = len(blocks)
        acc = x_scr[pl.ds(row0, TM), :].astype(F32)
        prev = None
        for j in range(NCH):
            g = _dot(xn, wg[j])
            u = _dot(xn, wu[j])
            h = (g * u).astype(BF)
            dn = _dot(h, wd[j])
            acc = acc + dn
            if j < ATTN_CHUNKS:
                mine = blocks[j * nb // ATTN_CHUNKS:(j + 1) * nb // ATTN_CHUNKS]
                evs = [g[0:R, 0:128], g[0:R, 384:512], u[0:R, 0:128], u[0:R, 384:512],
                       dn[0:R, 256:384], dn[0:R, 512:640], dn[0:R, 896:1024]]
                if len(mine) == 6:
                    evs = evs[0:5] + [dn[0:R, 768:896]]
                for e, r0 in zip(evs, mine):
                    tok = _bits(e) & zero
                    if prev is not None:
                        tok = tok | prev
                    prev = _attn_block(qkv, o_scr, row0, r0, tok, zero)
        acc = acc + _dot(o_scr[...], wo_bf[...])
        for p in range(OSPLIT):
            out_scr[pl.ds(row0, TM), p * OC:(p + 1) * OC] = acc[:, p * OC:(p + 1) * OC].astype(BF)
            out_copy(t, p).start()
        return carry

    qkv_copy(0).start()
    x_copy(0).start()
    for i in range(1, 6):
        qkv_copy(i).start()
    x_copy(1).start()
    wo_copy().start()
    x_copy(2).start()
    for j in range(NCH):
        for cp in ffn_copies(j):
            cp.start()
        if j + 3 < NT:
            x_copy(j + 3).start()

    first_tile()
    lax.fori_loop(1, NT, phase_a, 0)
    for j in range(NCH):
        for cp in ffn_copies(j):
            cp.wait()
    lax.fori_loop(0, NT, phase_b, 0)
    for t in range(NT):
        for p in range(OSPLIT):
            out_copy(t, p).wait()


@jax.jit
def pallas_parallel_sum__sliding_local_dilated__glu_gated_bilinear__prompt_kernel(
    A_x: jax.Array,
    A_wqkv: jax.Array,
    A_wo: jax.Array,
    B_x: jax.Array,
    B_w_gate: jax.Array,
    B_w_up: jax.Array,
    B_w_down: jax.Array,
):
    del B_x
    hbm = pl.BlockSpec(memory_space=pl.ANY)

    def packed(*shape):
        return pltpu.VMEM(shape[:-2] + (shape[-2] // 2, shape[-1]), U32)

    out = pl.pallas_call(
        _kernel,
        in_specs=[hbm] * 6,
        out_specs=hbm,
        out_shape=jax.ShapeDtypeStruct((S, D), BF),
        scratch_shapes=[
            packed(S, D), packed(S, D), packed(S, D),
            packed(TM, D), packed(TM, D),
            packed(6, KH, D), packed(D, D),
            packed(NCH, D, FC), packed(NCH, D, FC), packed(NCH, FC, D),
            packed(TM, D),
            packed(4, D, KH), packed(3, D, KH), packed(D, D),
            pltpu.VMEM((3, 8, S + HALO, 128), F32),
            pltpu.VMEM((4, H * PITCH + 32, 128), U32),
            pltpu.SemaphoreType.DMA((NSEM,)),
            pltpu.SemaphoreType.DMA((NT * OSPLIT,)),
        ],
        compiler_params=pltpu.CompilerParams(vmem_limit_bytes=120 << 20),
        name="fused_attn_glu",
    )(A_x.reshape(S, D), A_wqkv, A_wo, B_w_gate, B_w_up, B_w_down)
    return out.reshape(1, S, D)
```
